```python
import os as _os
_os.environ.setdefault("JAX_PLATFORMS", "cpu")
import jax
import jax.numpy as jnp

def _softmax(x, axis=-1):
    return jax.nn.softmax(x, axis=axis)
def _gelu(x):
    return jax.nn.gelu(x, approximate=True)
def _silu(x):
    return jax.nn.silu(x)
def _sigmoid(x):
    return jax.nn.sigmoid(x)
def _layernorm(x, axis=-1, eps=1e-5):
    m = jnp.mean(x, axis=axis, keepdims=True)
    v = jnp.var(x, axis=axis, keepdims=True)
    return (x - m) / jnp.sqrt(v + eps)
def _scatter_add(tgt, idx, src, axis=0):
    return tgt.at[idx].add(src)
def _segment_sum(src, seg, n):
    return jax.ops.segment_sum(src, seg, n)
class _Rng:
    def __init__(self, key):
        self._k = key
    def _next(self):
        self._k, sub = jax.random.split(self._k)
        return sub
    def normal(self, shape):
        return jax.random.normal(self._next(), shape, dtype=jnp.bfloat16)
    def randint(self, lo, hi, shape):
        return jax.random.randint(self._next(), shape, lo, hi, dtype=jnp.int32)
    def uniform(self, shape, lo=0.0, hi=1.0):
        return jax.random.uniform(self._next(), shape, jnp.bfloat16, lo, hi)
    def permutation(self, n):
        return jax.random.permutation(self._next(), n)


kernel_name = 'standalone__grn__sampling'

def setup_inputs():
    _rng = _Rng(jax.random.key(int.from_bytes(__import__("os").urandom(4), "little")))
    _w = (lambda a: (lambda t: t.astype(jnp.bfloat16) if jnp.issubdtype(t.dtype, jnp.floating) else t)(jnp.asarray(a)))
    B, S, D = 512, 32, 640
    return {
        "x": _w((lambda *s: _rng.normal(s) * 0.05)(B, S, D)),
        "g": _w((lambda *s: _rng.normal(s) * 0.1)(D) * 0.1),
        "b": _w((lambda *s: _rng.normal(s) * 0.1)(D) * 0.1),
    }

def reference(x, g, b):
    gx = jnp.sqrt((x * x).sum(axis=-2, keepdims=True))
    nx = gx / (gx.mean(axis=-1, keepdims=True) + 1e-6)
    return g * (x * nx) + b + x
```

```python
import jax
import jax.numpy as jnp
import jax.experimental.pallas as pl
import jax.experimental.pallas.tpu as pltpu


@jax.jit
def pallas_standalone__grn__sampling_kernel(
    x: jax.Array,
    g: jax.Array,
    b: jax.Array,
):
    B, S, D = x.shape
    bb = 64
    inner = 4

    def kernel_function(x_ref, g_ref, b_ref, o_ref):
        g2 = g_ref[...].astype(jnp.float32).reshape(1, D)
        b2 = b_ref[...].astype(jnp.float32).reshape(1, D)

        def step(j, c):
            for k in range(inner):
                i = j * inner + k
                xv = x_ref[i].astype(jnp.float32)
                gx = jnp.sqrt(jnp.sum(xv * xv, axis=0, keepdims=True))
                m = jnp.sum(gx, axis=-1, keepdims=True) * (1.0 / D) + 1e-6
                sc = g2 * (gx / m) + 1.0
                o_ref[i] = (xv * sc + b2).astype(o_ref.dtype)
            return c

        jax.lax.fori_loop(0, bb // inner, step, 0)

    return pl.pallas_call(
        kernel_function,
        grid=(B // bb,),
        in_specs=[
            pl.BlockSpec((bb, S, D), lambda i: (i, 0, 0)),
            pl.BlockSpec((D,), lambda i: (0,)),
            pl.BlockSpec((D,), lambda i: (0,)),
        ],
        out_specs=pl.BlockSpec((bb, S, D), lambda i: (i, 0, 0)),
        out_shape=jax.ShapeDtypeStruct((B, S, D), x.dtype),
        compiler_params=pltpu.CompilerParams(
            dimension_semantics=("parallel",), vmem_limit_bytes=64 * 2**20
        ),
    )(x, g, b)
```

```python
import jax
import jax.numpy as jnp
import jax.experimental.pallas as pl
import jax.experimental.pallas.tpu as pltpu

_STREAMS = 8


@jax.jit
def pallas_standalone__grn__sampling_kernel(
    x: jax.Array,
    g: jax.Array,
    b: jax.Array,
):
    B, S, D = x.shape
    K = _STREAMS
    N = B // K
    lead = N // 4
    shape = (K, N, S, D)

    def kernel_function(x_hbm, g_hbm, b_hbm, o_hbm, buf, g_buf, b_buf, sem_a, sem_b):
        def read(j0, n, sem):
            return pltpu.make_async_copy(
                x_hbm.at[:, pl.ds(j0, n)], buf.at[:, pl.ds(j0, n)], sem
            )

        def write(j):
            pltpu.make_async_copy(buf.at[:, j], o_hbm.at[:, j], sem_b).start()

        def loop(lo, hi, fn):
            def body(j, carry):
                fn(j)
                return carry

            jax.lax.fori_loop(lo, hi, body, 0)

        head = read(0, lead, sem_a)
        mid = read(lead, N - lead - 1, sem_b)
        tail = read(N - 1, 1, sem_a)
        g_cp = pltpu.make_async_copy(g_hbm, g_buf, sem_a)
        b_cp = pltpu.make_async_copy(b_hbm, b_buf, sem_a)
        head.start(priority=1)
        g_cp.start()
        b_cp.start()
        mid.start(priority=1)
        head.wait()
        g_cp.wait()
        b_cp.wait()
        tail.start(priority=1)

        g2 = g_buf[...].astype(jnp.float32).reshape(1, D)
        b2 = b_buf[...].astype(jnp.float32).reshape(1, D)

        def compute(j):
            for s in range(K):
                xv = buf[s, j].astype(jnp.float32)
                gx = jnp.sqrt(jnp.sum(xv * xv, axis=0, keepdims=True))
                m = jnp.sum(gx, axis=-1, keepdims=True) * (1.0 / D) + 1e-6
                sc = g2 * (gx / m) + 1.0
                buf[s, j] = (xv * sc + b2).astype(buf.dtype)

        def compute_and_write(j):
            compute(j)
            write(j)

        loop(0, lead, compute)
        mid.wait()
        loop(0, lead, write)
        loop(lead, N - 1, compute_and_write)
        tail.wait()
        compute_and_write(N - 1)
        pltpu.make_async_copy(buf, buf, sem_b).wait()

    out = pl.pallas_call(
        kernel_function,
        in_specs=[pl.BlockSpec(memory_space=pl.ANY)] * 3,
        out_specs=pl.BlockSpec(memory_space=pl.ANY),
        out_shape=jax.ShapeDtypeStruct(shape, x.dtype),
        scratch_shapes=[
            pltpu.VMEM(shape, x.dtype),
            pltpu.VMEM((D,), g.dtype),
            pltpu.VMEM((D,), b.dtype),
            pltpu.SemaphoreType.DMA,
            pltpu.SemaphoreType.DMA,
        ],
        compiler_params=pltpu.CompilerParams(vmem_limit_bytes=64 * 2**20),
    )(x.reshape(shape), g, b)
    return out.reshape(B, S, D)
```

```python
import jax
import jax.numpy as jnp
import jax.experimental.pallas as pl
import jax.experimental.pallas.tpu as pltpu

_EPS = 1e-6
_STREAMS = 8
_PIECES = 2
_TAIL = 9


@jax.jit
def pallas_standalone__grn__sampling_kernel(
    x: jax.Array,
    g: jax.Array,
    b: jax.Array,
):
    B, S, D = x.shape
    K = _STREAMS
    N = B // K
    lead = N // 4
    rows = S // _PIECES
    assert B % K == 0 and 0 < lead < N - _TAIL and S % (16 * _PIECES) == 0
    shape = (K, N, S, D)

    def kernel_function(x_hbm, g_hbm, b_hbm, o_hbm, x_buf, o_buf, g_buf, b_buf, bulk_sem):
        def read(idx, sem):
            return pltpu.make_async_copy(x_hbm.at[idx], x_buf.at[idx], sem)

        def start_write(j):
            for p in range(_PIECES):
                idx = (slice(None), j, pl.ds(p * rows, rows))
                pltpu.make_async_copy(o_buf.at[idx], o_hbm.at[idx], bulk_sem).start()

        def run(edge_sem):
            head = read((slice(None), pl.ds(0, lead)), edge_sem)
            g_copy = pltpu.make_async_copy(g_hbm, g_buf, edge_sem)
            b_copy = pltpu.make_async_copy(b_hbm, b_buf, edge_sem)
            middle = (
                read((pl.ds(0, K - 1), pl.ds(lead, N - lead)), bulk_sem),
                read((K - 1, pl.ds(lead, N - lead - _TAIL)), bulk_sem),
            )
            tail = read((K - 1, pl.ds(N - _TAIL, _TAIL)), edge_sem)

            head.start(priority=1)
            g_copy.start()
            b_copy.start()
            for copy in middle:
                copy.start(priority=1)
            head.wait()
            g_copy.wait()
            b_copy.wait()
            tail.start(priority=1)

            gamma = g_buf[...].astype(jnp.float32).reshape(1, D)
            beta = b_buf[...].astype(jnp.float32).reshape(1, D)

            def group(j, carry):
                @pl.when(j == lead)
                def _():
                    for copy in middle:
                        copy.wait()

                    def flush(i, carry):
                        start_write(i)
                        return carry

                    jax.lax.fori_loop(0, lead, flush, 0)

                @pl.when(j == N - _TAIL)
                def _():
                    tail.wait()

                for s in range(K):
                    xv = x_buf[s, j].astype(jnp.float32)
                    gx = jnp.sqrt(jnp.sum(xv * xv, axis=0, keepdims=True))
                    mean = jnp.sum(gx, axis=-1, keepdims=True) * (1.0 / D)
                    nx = gx / (mean + _EPS)
                    o_buf[s, j] = (xv * (gamma * nx + 1.0) + beta).astype(o_buf.dtype)

                @pl.when(j >= lead)
                def _():
                    start_write(j)

                return carry

            jax.lax.fori_loop(0, N, group, 0)

        pl.run_scoped(run, pltpu.SemaphoreType.DMA)
        pltpu.make_async_copy(o_buf, o_hbm, bulk_sem).wait()

    out = pl.pallas_call(
        kernel_function,
        in_specs=[pl.BlockSpec(memory_space=pl.ANY)] * 3,
        out_specs=pl.BlockSpec(memory_space=pl.ANY),
        out_shape=jax.ShapeDtypeStruct(shape, x.dtype),
        scratch_shapes=[
            pltpu.VMEM(shape, x.dtype),
            pltpu.VMEM(shape, x.dtype),
            pltpu.VMEM((D,), g.dtype),
            pltpu.VMEM((D,), b.dtype),
            pltpu.SemaphoreType.DMA,
        ],
        compiler_params=pltpu.CompilerParams(vmem_limit_bytes=64 * 2**20),
    )(x.reshape(shape), g, b)
    return out.reshape(B, S, D)
```
